```python
import os as _os
_os.environ.setdefault("JAX_PLATFORMS", "cpu")
import jax
import jax.numpy as jnp

def _softmax(x, axis=-1):
    return jax.nn.softmax(x, axis=axis)
def _gelu(x):
    return jax.nn.gelu(x, approximate=True)
def _silu(x):
    return jax.nn.silu(x)
def _sigmoid(x):
    return jax.nn.sigmoid(x)
def _layernorm(x, axis=-1, eps=1e-5):
    m = jnp.mean(x, axis=axis, keepdims=True)
    v = jnp.var(x, axis=axis, keepdims=True)
    return (x - m) / jnp.sqrt(v + eps)
def _scatter_add(tgt, idx, src, axis=0):
    return tgt.at[idx].add(src)
def _segment_sum(src, seg, n):
    return jax.ops.segment_sum(src, seg, n)
class _Rng:
    def __init__(self, key):
        self._k = key
    def _next(self):
        self._k, sub = jax.random.split(self._k)
        return sub
    def normal(self, shape):
        return jax.random.normal(self._next(), shape, dtype=jnp.bfloat16)
    def randint(self, lo, hi, shape):
        return jax.random.randint(self._next(), shape, lo, hi, dtype=jnp.int32)
    def uniform(self, shape, lo=0.0, hi=1.0):
        return jax.random.uniform(self._next(), shape, jnp.bfloat16, lo, hi)
    def permutation(self, n):
        return jax.random.permutation(self._next(), n)


kernel_name = 'concat_heads__linear_kernel_hedgehog__ssm_conv_s5__prompt'

def setup_inputs():
    _rng = _Rng(jax.random.key(int.from_bytes(__import__("os").urandom(4), "little")))
    _w = (lambda a: (lambda t: t.astype(jnp.bfloat16) if jnp.issubdtype(t.dtype, jnp.floating) else t)(jnp.asarray(a)))
    def _A_setup():
        B, S, D, H = 1, 2048, 640, 32
        Dh = D // H
        return {
            "x": _w((lambda *s: _rng.normal(s) * 0.4)(B, S, D)),
            "wqkv": _w((lambda *s: _rng.normal(s) * 0.4)(D, 3 * D)),
            "w_phi": _w((lambda *s: _rng.normal(s) * 0.4)(H, Dh, Dh) * (Dh ** -0.5)),
            "wo": _w((lambda *s: _rng.normal(s) * 0.05)(D, D)),
        }
    _A_in = _A_setup()

    def _B_setup():
        B, S, D = 1, 2048, 640
        P = D
        Lambda_re = -0.5 * jnp.exp((lambda *s: _rng.normal(s) * 0.8)(P))
        Lambda_im = (lambda *s: _rng.normal(s) * 0.8)(P) * 1.0
        B_re = (lambda *s: _rng.normal(s) * 0.8)(P, D) * (D ** -0.5)
        B_im = (lambda *s: _rng.normal(s) * 0.8)(P, D) * (D ** -0.5)
        C_re = (lambda *s: _rng.normal(s) * 0.8)(D, P) * (P ** -0.5)
        C_im = (lambda *s: _rng.normal(s) * 0.8)(D, P) * (P ** -0.5)
        log_dt = (lambda *s: _rng.normal(s) * 0.8)(P) * 0.3 - 2.0
        Dskip = (lambda *s: _rng.normal(s) * 0.8)(D)
        return {
            "x": _w((lambda *s: _rng.normal(s) * 0.05)(B, S, D)),
            "Lambda_re": _w(Lambda_re),
            "Lambda_im": _w(Lambda_im),
            "B_re": _w(B_re),
            "B_im": _w(B_im),
            "C_re": _w(C_re),
            "C_im": _w(C_im),
            "log_dt": _w(log_dt),
            "Dskip": _w(Dskip),
        }
    _B_in = _B_setup()

    return {
        "A_x": _A_in["x"],
        "A_wqkv": _A_in["wqkv"],
        "A_w_phi": _A_in["w_phi"],
        "A_wo": _A_in["wo"],
        "B_x": _B_in["x"],
        "B_Lambda_re": _B_in["Lambda_re"],
        "B_Lambda_im": _B_in["Lambda_im"],
        "B_B_re": _B_in["B_re"],
        "B_B_im": _B_in["B_im"],
        "B_C_re": _B_in["C_re"],
        "B_C_im": _B_in["C_im"],
        "B_log_dt": _B_in["log_dt"],
        "B_Dskip": _B_in["Dskip"],
    }

def reference(A_x, A_wqkv, A_w_phi, A_wo, B_x, B_Lambda_re, B_Lambda_im, B_B_re, B_B_im, B_C_re, B_C_im, B_log_dt, B_Dskip):
    def _A_ref(x, wqkv, w_phi, wo):
        B, S, D = x.shape
        H = 32; Dh = D // H
        qkv = (lambda x, *d: x.transpose(*d))((x @ wqkv).reshape(B, S, 3, H, Dh), 2, 0, 3, 1, 4)
        q, k, v = qkv[0], qkv[1], qkv[2]
        pq = jnp.einsum("bhsd,hdf->bhsf", q, w_phi)
        pk = jnp.einsum("bhsd,hdf->bhsf", k, w_phi)
        phi_q = jnp.concatenate([_softmax(pq, axis=-1), _softmax(-pq, axis=-1)], axis=-1)
        phi_k = jnp.concatenate([_softmax(pk, axis=-1), _softmax(-pk, axis=-1)], axis=-1)
        kv = jnp.einsum("bhsf,bhsd->bhfd", phi_k, v)
        z  = jnp.einsum("bhsf->bhf", phi_k)
        num = jnp.einsum("bhqf,bhfd->bhqd", phi_q, kv)
        den = jnp.einsum("bhqf,bhf->bhq", phi_q, z)[..., None] + 1e-6
        o = num / den
        return (lambda x, *d: x.transpose(*d))(o, 0, 2, 1, 3).reshape(B, S, D) @ wo

    def _B_ref(x, Lambda_re, Lambda_im, B_re, B_im, C_re, C_im, log_dt, Dskip):
        Bsz, L, H = x.shape
        Lam = Lambda_re + 1j * Lambda_im
        Bmat = B_re + 1j * B_im
        Cmat = C_re + 1j * C_im
        dt = jnp.exp(log_dt)
        Lam_bar = jnp.exp(dt * Lam)
        B_bar = ((Lam_bar - 1.0) / Lam)[:, None] * Bmat
        Bu = jnp.einsum("bld,pd->blp", x + 0j, B_bar)
        h = jnp.zeros_like(Bu[:, 0, :])
        hs = []
        for t in range(L):
            h = Lam_bar[None, :] * h + Bu[:, t, :]
            hs.append(h)
        hseq = jnp.stack(hs, 1)
        y = 2.0 * jnp.einsum("blp,dp->bld", hseq, Cmat).real + x * Dskip[None, None, :]
        return y

    a = _A_ref(A_x, A_wqkv, A_w_phi, A_wo)
    b = _B_ref(B_x, B_Lambda_re, B_Lambda_im, B_B_re, B_B_im, B_C_re, B_C_im, B_log_dt, B_Dskip)
    return jnp.concatenate([a, b], axis=-1)
```

```python
import numpy as np
import jax
import jax.numpy as jnp
from jax import lax
import jax.experimental.pallas as pl
import jax.experimental.pallas.tpu as pltpu

S = 2048
D = 640
H = 32
DH = 20
NG = 4
GR = 160
LT = D // 128
TA = 512
TQ = 1024
TB = 1024
NCA = S // TA
NCB = S // TB
NCQ = S // TQ
PR = 40
NP = 16
NSUB = 8
BLK = 64

LOG2E = float(np.log2(np.e))

F32 = jnp.float32
BF16 = jnp.bfloat16
U32 = jnp.uint32

NT = (((1,), (1,)), ((), ()))
NN = (((1,), (0,)), ((), ()))
TN = (((0,), (0,)), ((), ()))


UNROLL = False


def _loop(n, body):
    if UNROLL:
        for c in range(n):
            body(c, 0)
    else:
        lax.fori_loop(0, n, body, 0)


def _rows(c, t):
    if isinstance(c, int):
        return pl.ds(c * t, t)
    return pl.ds(pl.multiple_of(c * t, t), t)


def _when(cond):
    if isinstance(cond, bool):
        return (lambda f: f()) if cond else (lambda f: None)
    return pl.when(cond)


def _dot(a, b, dims):
    return lax.dot_general(a, b, dims, preferred_element_type=F32)


def _cmul(ar, ai, br, bi):
    return ar * br - ai * bi, ar * bi + ai * br


def _pack(x):
    return pltpu.bitcast(x.astype(BF16), U32)


def _pack2(even, odd):
    return pltpu.pack_elementwise([even, odd], packed_dtype=BF16)


def _unpack2(w):
    return tuple(pltpu.unpack_elementwise(w, index=i, packed_dtype=BF16, unpacked_dtype=F32)
                 for i in range(2))


def _unpack(x):
    return pltpu.bitcast(x, BF16)


def _recip(x):
    return pl.reciprocal(x, full_range=False)


def _allreduce(x, op):
    x = op(x, pltpu.roll(x, 2, 0))
    return op(x, pltpu.roll(x, 4, 0))


def _feature_map(p):
    t = p.shape[1]
    p3 = p.reshape(5, 8, t)
    mx = _allreduce(jnp.max(p3, axis=0), jnp.maximum)
    mn = _allreduce(jnp.min(p3, axis=0), jnp.minimum)
    e1 = jnp.exp2(p3 - mx[None])
    e2 = jnp.exp2(mn[None] - p3)
    r1 = _recip(_allreduce(jnp.sum(e1, axis=0), jnp.add))
    r2 = _recip(_allreduce(jnp.sum(e2, axis=0), jnp.add))
    phi = jnp.concatenate([e1 * r1[None], e2 * r2[None]], axis=0)
    return phi.reshape(2 * PR, t).astype(BF16)


def _kernel(xa_hbm, wqkv_hbm, wphi_hbm, wo_hbm, xb_hbm, lre_hbm, lim_hbm, bre_hbm, bim_hbm,
            cre_hbm, cim_hbm, ldt_hbm, dsk_hbm,
            out_hbm,
            xa, xb, wqkv, wo, bre, bim, cre, cim, wphi, vecs,
            wall, wt, cp, lam, kv, kvm, xperm, ubuf, hbuf, carry, ob, oa,
            sem_w, sem_xa, sem_xb, sem_o):
    cp_in = pltpu.make_async_copy
    xa_hbm, wqkv_hbm, wo_hbm, xb_hbm, bre_hbm, bim_hbm, cre_hbm, cim_hbm = (
        r.bitcast(U32) for r in (xa_hbm, wqkv_hbm, wo_hbm, xb_hbm, bre_hbm, bim_hbm, cre_hbm, cim_hbm))
    small = [
        cp_in(wphi_hbm, wphi, sem_w.at[0]),
        cp_in(lre_hbm, vecs[0], sem_w.at[1]),
        cp_in(lim_hbm, vecs[1], sem_w.at[7]),
        cp_in(ldt_hbm, vecs[2], sem_w.at[8]),
        cp_in(dsk_hbm, vecs[3], sem_w.at[9]),
    ]
    wk_cp = cp_in(wqkv_hbm.at[:, pl.ds(D, D)], wqkv.at[1], sem_w.at[2])
    wv_cp = cp_in(wqkv_hbm.at[:, pl.ds(2 * D, D)], wqkv.at[2], sem_w.at[3])
    wq_cp = cp_in(wqkv_hbm.at[:, pl.ds(0, D)], wqkv.at[0], sem_w.at[4])
    bre_cp = cp_in(bre_hbm, bre, sem_w.at[5])
    bim_cp = cp_in(bim_hbm, bim, sem_w.at[10])
    wo_cp = cp_in(wo_hbm, wo, sem_w.at[6])
    cre_cp = cp_in(cre_hbm, cre, sem_w.at[11])
    cim_cp = cp_in(cim_hbm, cim, sem_w.at[12])

    def xa_cp(c):
        r = _rows(c, TA // 2)
        return cp_in(xa_hbm.at[r, :], xa.at[r, :], sem_xa.at[c])

    def xb_cp(c):
        r = _rows(c, TB // 2)
        return [cp_in(xb_hbm.at[r, pl.ds(128 * lt, 128)], xb.at[lt, r, :], sem_xb.at[c])
                for lt in range(LT)]

    def ob_cp(c, slot):
        return cp_in(ob.at[slot], out_hbm.at[_rows(c, TB), pl.ds(D, D)], sem_o.at[0])

    def oa_cp(c, slot, j):
        ts = TQ // NSUB
        if isinstance(c, int):
            r = pl.ds(c * TQ + j * ts, ts)
        else:
            r = pl.ds(pl.multiple_of(c * TQ + j * ts, ts), ts)
        return cp_in(oa.at[slot, pl.ds(j * ts, ts), :], out_hbm.at[r, pl.ds(0, D)], sem_o.at[1])

    for c in small:
        c.start()
    wk_cp.start()

    small[0].wait()
    wv_cp.start()
    xa_cp(0).start()
    for e in range(DH):
        t = jnp.pad(wphi[e].astype(F32), ((0, 128 - DH), (0, 128 - H))).T
        wall[pl.ds(e, H, stride=DH), :] = t[:H]
    def logical(r):
        return (r // 16) * 16 + 2 * (r % 8) + (r % 16) // 8

    ri = logical(lax.broadcasted_iota(jnp.int32, (GR, 128), 0))
    ci = lax.broadcasted_iota(jnp.int32, (GR, 128), 1)
    et = jnp.where((ri % PR) // 2 == ci, 1.0, 0.0).astype(BF16)
    r2 = logical(lax.broadcasted_iota(jnp.int32, (GR, 256), 0))
    c2 = lax.broadcasted_iota(jnp.int32, (GR, 256), 1)
    bdt = []
    for g in range(NG):
        ws = 128 * ((GR * g) // 128)
        keep = ((c2 + ws) // DH) == (8 * g + 2 * (r2 // PR) + r2 % 2)
        full = _dot(et, wall[pl.ds(ws, 256), :].astype(BF16), NT)
        bdt.append(jnp.where(keep, full, 0.0).astype(BF16))

    def fold(j, g):
        ws = 128 * ((GR * g) // 128)
        w = _dot(bdt[g], _unpack(wqkv[j, :, pl.ds(ws, 256)]), NT)
        w = w * LOG2E
        packed = []
        for r in range(0, GR, 16):
            packed.append(_pack2(w[r:r + 8], w[r + 8:r + 16]))
            wt[j, pl.ds((GR * g + r) // 2, 8), :] = packed[-1]
        return packed

    def wrows(j, g):
        return _unpack(wt[j, pl.ds(GR // 2 * g, GR // 2), :])

    for c in small[1:]:
        c.wait()
    l_re = vecs[0][...].reshape(1, D).astype(F32)
    l_im = vecs[1][...].reshape(1, D).astype(F32)
    dt = jnp.exp(vecs[2][...].reshape(1, D).astype(F32)).astype(BF16).astype(F32)
    mag = jnp.exp(dt * l_re)
    ang = dt * l_im
    a_re = mag * jnp.cos(ang)
    a_im = mag * jnp.sin(ang)
    den = l_re * l_re + l_im * l_im
    n_re = a_re - 1.0
    k_re = (n_re * l_re + a_im * l_im) / den
    k_im = (a_im * l_re - n_re * l_im) / den
    pw = (a_re, a_im)
    pows = [pw]
    for _ in range(5):
        pw = _cmul(pw[0], pw[1], pw[0], pw[1])
        pows.append(pw)
    for i, k in enumerate((0, 3, 4, 5)):
        lam[2 * i] = jnp.broadcast_to(pows[k][0], (8, D))
        lam[2 * i + 1] = jnp.broadcast_to(pows[k][1], (8, D))
    lam[8] = jnp.broadcast_to(vecs[3][...].reshape(1, D).astype(F32), (8, D))
    lam[9] = jnp.broadcast_to(2.0 * k_re, (8, D))
    lam[10] = jnp.broadcast_to(2.0 * k_im, (8, D))
    carry[...] = jnp.zeros(carry.shape, F32)
    kv[...] = jnp.zeros(kv.shape, F32)

    wk_cp.wait()
    for g in range(NG):
        fold(1, g)
    wv_cp.wait()
    wt[2] = _pack(_unpack(wqkv[2]).astype(F32).T)

    def phase1(c, _):
        @_when(c + 1 < NCA)
        def _():
            xa_cp(c + 1).start()

        @_when(c == 0)
        def _():
            wq_cp.start()
            cre_cp.start()
            cim_cp.start()

        @_when(c == NCA // 2)
        def _():
            bre_cp.start()
            bim_cp.start()
            for d in xb_cp(0):
                d.start()

        xa_cp(c).wait()
        xc = _unpack(xa[_rows(c, TA // 2), :])
        ones = jnp.ones((8, TA), F32)
        for g in range(NG):
            pk = _dot(wrows(1, g), xc, NT)
            vt = _dot(wrows(2, g), xc, NT)
            for j in range(4):
                phi = _feature_map(pk[PR * j:PR * (j + 1)])
                lhs = jnp.concatenate([vt[PR * j:PR * (j + 1)], ones], axis=0).astype(BF16)
                kv[4 * g + j] += _dot(lhs, phi, NT)
        return 0

    _loop(NCA, phase1)

    wq_cp.wait()
    cre_cp.wait()
    cim_cp.wait()
    k2r = lam[9]
    k2i = lam[10]
    kni = -k2i
    rr = lax.broadcasted_iota(jnp.int32, (48, 2 * PR), 0)
    cc = lax.broadcasted_iota(jnp.int32, (48, 2 * PR), 1)
    diag = jnp.where(rr < PR, rr // DH, (rr - PR) // 4) == (cc % 2)
    zero = pltpu.bitcast(carry[0], U32)
    for g in range(NG):
        packed = fold(0, g)
        for i, r in enumerate(range(GR * g, GR * (g + 1), 16)):
            tie = packed[i] & zero
            c_r = _unpack2(cre[pl.ds(r // 2, 8), :] | tie)
            c_i = _unpack2(cim[pl.ds(r // 2, 8), :] | tie)
            cp[pl.ds(r // 2, 8), 0:D] = _pack2(*[c_r[i] * k2r - c_i[i] * k2i for i in range(2)])
            cp[pl.ds(r // 2, 8), D:2 * D] = _pack2(*[c_r[i] * kni - c_i[i] * k2r for i in range(2)])
        for j in range(4 * g, 4 * g + 4):
            kvm[j] = _pack(jnp.where(diag, kv[j], 0.0))
    bre_cp.wait()
    bim_cp.wait()

    sub = lax.broadcasted_iota(jnp.int32, (8, 128), 0)

    def phase_b(c, _):
        slot = c

        @_when(c + 1 < NCB)
        def _():
            for d in xb_cp(c + 1):
                d.start()

        @_when(c == 0)
        def _():
            wo_cp.start()

        whole = xb.at[:, _rows(c, TB // 2), :]
        cp_in(whole, whole, sem_xb.at[c]).wait()

        base = c * (TB // 2)
        for b in range(TB // BLK):
            for lt in range(LT):
                pieces = []
                for j in range(4):
                    pieces.extend(_unpack2(xb[lt, pl.ds(base + 32 * b + j, 8, stride=4), :]))
                xperm[pl.ds(BLK // 2 * b, BLK // 2), 128 * lt:128 * (lt + 1)] = (
                    _pack(jnp.concatenate(pieces, axis=0)))
        xp = _unpack(xperm[...])
        ubuf[0] = _dot(xp, _unpack(bre[...]), NT)
        ubuf[1] = _dot(xp, _unpack(bim[...]), NT)
        for lt in range(LT):
            ls = slice(128 * lt, 128 * (lt + 1))
            l1 = (lam[0, :, ls], lam[1, :, ls])
            l8 = [(lam[2, :, ls], lam[3, :, ls]), (lam[4, :, ls], lam[5, :, ls]), (lam[6, :, ls], lam[7, :, ls])]
            pr, pi = carry[0, :, ls], carry[1, :, ls]
            for b in range(TB // BLK):
                def u(i):
                    return (ubuf[0, pl.ds(BLK * b + 8 * i, 8), ls], ubuf[1, pl.ds(BLK * b + 8 * i, 8), ls])
                hr, hi = u(0)
                for i in range(1, 8):
                    hr, hi = _cmul(l1[0], l1[1], hr, hi)
                    ur, ui = u(i)
                    hr, hi = hr + ur, hi + ui
                sr = jnp.where(sub == 0, pltpu.roll(pr, 1, 0), pltpu.roll(hr, 1, 0))
                si = jnp.where(sub == 0, pltpu.roll(pi, 1, 0), pltpu.roll(hi, 1, 0))
                for k, sh in enumerate((1, 2, 4)):
                    tr = jnp.where(sub >= sh, pltpu.roll(sr, sh, 0), 0.0)
                    ti = jnp.where(sub >= sh, pltpu.roll(si, sh, 0), 0.0)
                    tr, ti = _cmul(l8[k][0], l8[k][1], tr, ti)
                    sr, si = sr + tr, si + ti
                hr, hi = sr, si
                hs = []
                for i in range(8):
                    hr, hi = _cmul(l1[0], l1[1], hr, hi)
                    ur, ui = u(i)
                    hr, hi = hr + ur, hi + ui
                    hs.append((hr, hi))
                pr, pi = hr, hi
                for j in range(4):
                    hbuf[lt, pl.ds(32 * b + j, 8, stride=4), :] = _pack2(hs[2 * j][0], hs[2 * j + 1][0])
                    hbuf[LT + lt, pl.ds(32 * b + j, 8, stride=4), :] = _pack2(hs[2 * j][1], hs[2 * j + 1][1])
            carry[0, :, ls] = pr
            carry[1, :, ls] = pi
        hcat = jnp.concatenate([_unpack(hbuf[k]) for k in range(2 * LT)], axis=1)
        xc = jnp.concatenate([_unpack(xb[lt, _rows(c, TB // 2), :]) for lt in range(LT)], axis=1)
        ob[slot] = _dot(hcat, _unpack(cp[...]), NT) + xc.astype(F32) * lam[8, 0:1, :]
        ob_cp(c, slot).start()
        return 0

    _loop(NCB, phase_b)

    wo_cp.wait()

    def phase2(c, _):
        slot = c

        xq = _unpack(xa[_rows(c, TQ // 2), :])
        subt = lax.broadcasted_iota(jnp.int32, (8, TQ), 0)
        ots = []
        for g in range(NG):
            pq = _dot(wrows(0, g), xq, NT)
            for j in range(4):
                phi = _feature_map(pq[PR * j:PR * (j + 1)])
                nd = _dot(_unpack(kvm[4 * g + j]), phi, NN)
                rd = _recip(nd[PR:] + 1e-6)
                sw = pltpu.roll(rd, 4, 0)
                r0 = jnp.where(subt < 4, rd, sw)
                r1 = jnp.where(subt < 4, sw, rd)
                ots.append(nd[:PR] * jnp.concatenate([r0, r0, rd, r1, r1], axis=0))
        ot = jnp.concatenate(ots, axis=0)
        ts = TQ // NSUB
        for j in range(NSUB):
            a = _dot(ot[:, j * ts:(j + 1) * ts].T.astype(BF16), _unpack(wo[...]), NN)
            oa[slot, pl.ds(j * ts, ts), :] = a.astype(BF16).astype(F32)
            oa_cp(c, slot, j).start()
        return 0

    _loop(NCQ, phase2)

    for c in range(NCB):
        ob_cp(c, c).wait()
    for c in range(NCQ):
        for j in range(NSUB):
            oa_cp(c, c, j).wait()


@jax.jit
def pallas_concat_heads__linear_kernel_hedgehog__ssm_conv_s5__prompt_kernel(
    A_x: jax.Array,
    A_wqkv: jax.Array,
    A_w_phi: jax.Array,
    A_wo: jax.Array,
    B_x: jax.Array,
    B_Lambda_re: jax.Array,
    B_Lambda_im: jax.Array,
    B_B_re: jax.Array,
    B_B_im: jax.Array,
    B_C_re: jax.Array,
    B_C_im: jax.Array,
    B_log_dt: jax.Array,
    B_Dskip: jax.Array,
):
    any_spec = pl.BlockSpec(memory_space=pl.ANY)
    vm = pltpu.VMEM
    scratch = [
        vm((S // 2, D), U32),
        vm((LT, S // 2, 128), U32),
        vm((3, D // 2, D), U32),
        vm((D // 2, D), U32),
        vm((D // 2, D), U32),
        vm((D // 2, D), U32),
        vm((D // 2, D), U32),
        vm((D // 2, D), U32),
        vm((DH, DH, H), BF16),
        [vm((D,), BF16) for _ in range(4)],
        vm((D, 128), F32),
        vm((3, D // 2, D), U32),
        vm((D // 2, 2 * D), U32),
        vm((11, 8, D), F32),
        vm((NP, 48, 2 * PR), F32),
        vm((NP, 24, 2 * PR), U32),
        vm((TB // 2, D), U32),
        vm((2, TB, D), F32),
        vm((2 * LT, TB // 2, 128), U32),
        vm((2, 8, D), F32),
        vm((NCB, TB, D), F32),
        vm((NCQ, TQ, D), F32),
        pltpu.SemaphoreType.DMA((13,)),
        pltpu.SemaphoreType.DMA((NCA,)),
        pltpu.SemaphoreType.DMA((NCB,)),
        pltpu.SemaphoreType.DMA((2,)),
    ]
    out = pl.pallas_call(
        _kernel,
        out_shape=jax.ShapeDtypeStruct((S, 2 * D), F32),
        in_specs=[any_spec] * 13,
        out_specs=any_spec,
        scratch_shapes=scratch,
        compiler_params=pltpu.CompilerParams(vmem_limit_bytes=100 * 1024 * 1024, flags={"XLA_TPU_RESCHEDULE_DMA_DONES": True}),
    )(A_x.reshape(S, D), A_wqkv, A_w_phi.transpose(1, 2, 0), A_wo, B_x.reshape(S, D), B_Lambda_re, B_Lambda_im,
      B_B_re, B_B_im, B_C_re, B_C_im, B_log_dt, B_Dskip)
    return out.reshape(1, S, 2 * D)
```

```python
import numpy as np
import jax
import jax.numpy as jnp
from jax import lax
import jax.experimental.pallas as pl
import jax.experimental.pallas.tpu as pltpu

S = 2048
D = 640
H = 32
DH = 20
NG = 4
GR = 160
LT = D // 128
TA = 512
TQ = 1024
TB = 1024
NCA = S // TA
NCB = S // TB
NCQ = S // TQ
PR = 40
NP = 16
NSUB = 8
BLK = 64

LOG2E = float(np.log2(np.e))

F32 = jnp.float32
BF16 = jnp.bfloat16
U32 = jnp.uint32

NT = (((1,), (1,)), ((), ()))
NN = (((1,), (0,)), ((), ()))


def _rows(c, t):
    if isinstance(c, int):
        return pl.ds(c * t, t)
    return pl.ds(pl.multiple_of(c * t, t), t)


def _when(cond):
    if isinstance(cond, bool):
        return (lambda f: f()) if cond else (lambda f: None)
    return pl.when(cond)


def _dot(a, b, dims):
    return lax.dot_general(a, b, dims, preferred_element_type=F32)


def _cmul(ar, ai, br, bi):
    return ar * br - ai * bi, ar * bi + ai * br


def _pack(x):
    return pltpu.bitcast(x.astype(BF16), U32)


def _pack2(even, odd):
    return pltpu.pack_elementwise([even, odd], packed_dtype=BF16)


def _unpack2(w):
    return tuple(pltpu.unpack_elementwise(w, index=i, packed_dtype=BF16, unpacked_dtype=F32)
                 for i in range(2))


def _unpack(x):
    return pltpu.bitcast(x, BF16)


def _recip(x):
    return pl.reciprocal(x, full_range=False)


def _allreduce(x, op):
    x = op(x, pltpu.roll(x, 2, 0))
    return op(x, pltpu.roll(x, 4, 0))


def _feature_map(p):
    t = p.shape[1]
    p3 = p.reshape(5, 8, t)
    mx = _allreduce(jnp.max(p3, axis=0), jnp.maximum)
    mn = _allreduce(jnp.min(p3, axis=0), jnp.minimum)
    e1 = jnp.exp2(p3 - mx[None])
    e2 = jnp.exp2(mn[None] - p3)
    r1 = _recip(_allreduce(jnp.sum(e1, axis=0), jnp.add))
    r2 = _recip(_allreduce(jnp.sum(e2, axis=0), jnp.add))
    phi = jnp.concatenate([e1 * r1[None], e2 * r2[None]], axis=0)
    return phi.reshape(2 * PR, t).astype(BF16)


def _kernel(xa_hbm, wqkv_hbm, wphi_hbm, wo_hbm, xb_hbm, lre_hbm, lim_hbm, bre_hbm, bim_hbm,
            cre_hbm, cim_hbm, ldt_hbm, dsk_hbm,
            out_hbm,
            xa, xb, wqkv, wo, bre, bim, cre, cim, wphi, vecs,
            wall, wt, cp, lam, kv, kvm, xperm, ubuf, hbuf, carry, ob, oa,
            sem_w, sem_wk, sem_xa, sem_xb, sem_o):
    cp_in = pltpu.make_async_copy
    xa_hbm, wqkv_hbm, wo_hbm, xb_hbm, bre_hbm, bim_hbm, cre_hbm, cim_hbm = (
        r.bitcast(U32) for r in (xa_hbm, wqkv_hbm, wo_hbm, xb_hbm, bre_hbm, bim_hbm, cre_hbm, cim_hbm))
    small = [
        cp_in(wphi_hbm, wphi, sem_w.at[0]),
        cp_in(lre_hbm, vecs[0], sem_w.at[1]),
        cp_in(lim_hbm, vecs[1], sem_w.at[7]),
        cp_in(ldt_hbm, vecs[2], sem_w.at[8]),
        cp_in(dsk_hbm, vecs[3], sem_w.at[9]),
    ]
    wk_parts = ((0, 3), (3, 5))
    wk_cp = [cp_in(wqkv_hbm.at[pl.ds(64 * a, 64 * (b - a)), pl.ds(D, D)],
                   wqkv.at[1, pl.ds(64 * a, 64 * (b - a)), :], sem_wk.at[i])
             for i, (a, b) in enumerate(wk_parts)]
    wv_cp = cp_in(wqkv_hbm.at[:, pl.ds(2 * D, D)], wqkv.at[2], sem_w.at[3])
    wq_cp = cp_in(wqkv_hbm.at[:, pl.ds(0, D)], wqkv.at[0], sem_w.at[4])
    bre_cp = cp_in(bre_hbm, bre, sem_w.at[5])
    bim_cp = cp_in(bim_hbm, bim, sem_w.at[10])
    wo_cp = cp_in(wo_hbm, wo, sem_w.at[6])
    cre_cp = cp_in(cre_hbm, cre, sem_w.at[11])
    cim_cp = cp_in(cim_hbm, cim, sem_w.at[12])

    def xa_cp(c):
        r = _rows(c, TA // 2)
        return cp_in(xa_hbm.at[r, :], xa.at[r, :], sem_xa.at[c])

    def xb_cp(c):
        r = _rows(c, TB // 2)
        return [cp_in(xb_hbm.at[r, pl.ds(128 * lt, 128)], xb.at[lt, r, :], sem_xb.at[c])
                for lt in range(LT)]

    def ob_cp(c, slot):
        return cp_in(ob.at[slot], out_hbm.at[_rows(c, TB), pl.ds(D, D)], sem_o.at[0])

    def oa_cp(c, slot, j):
        ts = TQ // NSUB
        if isinstance(c, int):
            r = pl.ds(c * TQ + j * ts, ts)
        else:
            r = pl.ds(pl.multiple_of(c * TQ + j * ts, ts), ts)
        return cp_in(oa.at[slot, pl.ds(j * ts, ts), :], out_hbm.at[r, pl.ds(0, D)], sem_o.at[1])

    for c in small:
        c.start()
    for d in wk_cp:
        d.start()

    def logical(r):
        return (r // 16) * 16 + 2 * (r % 8) + (r % 16) // 8

    ri = logical(lax.broadcasted_iota(jnp.int32, (GR, 128), 0))
    ci = lax.broadcasted_iota(jnp.int32, (GR, 128), 1)
    et = jnp.where((ri % PR) // 2 == ci, 1.0, 0.0).astype(BF16)
    r2 = logical(lax.broadcasted_iota(jnp.int32, (GR, 256), 0))
    c2 = lax.broadcasted_iota(jnp.int32, (GR, 256), 1)
    keeps = [((c2 + 128 * ((GR * g) // 128)) // DH) == (8 * g + 2 * (r2 // PR) + r2 % 2)
             for g in range(NG)]
    kv[...] = jnp.zeros(kv.shape, F32)
    carry[...] = jnp.zeros(carry.shape, F32)
    small[0].wait()
    xa_cp(0).start()
    wv_cp.start()
    for e in range(DH):
        t = jnp.pad(wphi[e].astype(F32), ((0, 128 - DH), (0, 128 - H))).T
        wall[pl.ds(e, H, stride=DH), :] = t[:H]
    bdt = []
    for g in range(NG):
        ws = 128 * ((GR * g) // 128)
        keep = keeps[g]
        full = _dot(et, wall[pl.ds(ws, 256), :].astype(BF16), NT)
        bdt.append(jnp.where(keep, full, 0.0).astype(BF16))

    def fold(j, g):
        ws = 128 * ((GR * g) // 128)
        w = _dot(bdt[g], _unpack(wqkv[j, :, pl.ds(ws, 256)]), NT)
        w = w * LOG2E
        packed = []
        for r in range(0, GR, 16):
            packed.append(_pack2(w[r:r + 8], w[r + 8:r + 16]))
            wt[j, pl.ds((GR * g + r) // 2, 8), :] = packed[-1]
        return packed

    def wrows(j, g):
        return _unpack(wt[j, pl.ds(GR // 2 * g, GR // 2), :])

    for i, (a, b) in enumerate(wk_parts):
        wk_cp[i].wait()
        for g in range(NG):
            ws = 128 * ((GR * g) // 128)
            w = _dot(bdt[g], _unpack(wqkv[1, pl.ds(64 * a, 64 * (b - a)), pl.ds(ws, 256)]), NT) * LOG2E
            for r in range(0, GR, 16):
                wt[1, pl.ds((GR * g + r) // 2, 8), pl.ds(128 * a, 128 * (b - a))] = (
                    _pack2(w[r:r + 8], w[r + 8:r + 16]))

    def key_features(xc, g):
        pk = _dot(wrows(1, g), xc, NT)
        return [_feature_map(pk[PR * j:PR * (j + 1)]) for j in range(4)]

    def accumulate_kv(xc, g, phis):
        vt = _dot(wrows(2, g), xc, NT)
        ones = jnp.ones((8, TA), F32)
        for j in range(4):
            lhs = jnp.concatenate([vt[PR * j:PR * (j + 1)], ones], axis=0).astype(BF16)
            kv[4 * g + j] += _dot(lhs, phis[j], NT)

    xa_cp(0).wait()
    xa_cp(1).start()
    xc0 = _unpack(xa[pl.ds(0, TA // 2), :])
    phis0 = [key_features(xc0, g) for g in range(NG)]
    wv_cp.wait()
    for c in small[1:]:
        c.wait()
    wt[2] = _pack(_unpack(wqkv[2]).astype(F32).T)
    for g in range(NG):
        accumulate_kv(xc0, g, phis0[g])

    l_re = vecs[0][...].reshape(1, D).astype(F32)
    l_im = vecs[1][...].reshape(1, D).astype(F32)
    dt = jnp.exp(vecs[2][...].reshape(1, D).astype(F32)).astype(BF16).astype(F32)
    mag = jnp.exp(dt * l_re)
    ang = dt * l_im
    a_re = mag * jnp.cos(ang)
    a_im = mag * jnp.sin(ang)
    den = l_re * l_re + l_im * l_im
    n_re = a_re - 1.0
    k_re = (n_re * l_re + a_im * l_im) / den
    k_im = (a_im * l_re - n_re * l_im) / den
    pw = (a_re, a_im)
    pows = [pw]
    for _ in range(5):
        pw = _cmul(pw[0], pw[1], pw[0], pw[1])
        pows.append(pw)
    for i, k in enumerate((0, 3, 4, 5)):
        lam[2 * i] = jnp.broadcast_to(pows[k][0], (8, D))
        lam[2 * i + 1] = jnp.broadcast_to(pows[k][1], (8, D))
    lam[8] = jnp.broadcast_to(vecs[3][...].reshape(1, D).astype(F32), (8, D))
    lam[9] = jnp.broadcast_to(2.0 * k_re, (8, D))
    lam[10] = jnp.broadcast_to(2.0 * k_im, (8, D))

    def phase1(c, _):
        @_when(c + 1 < NCA)
        def _():
            xa_cp(c + 1).start()

        @_when(c == 1)
        def _():
            wq_cp.start()
            cre_cp.start()
            cim_cp.start()

        @_when(c == 2)
        def _():
            bre_cp.start()
            bim_cp.start()
            for d in xb_cp(0):
                d.start()

        xa_cp(c).wait()
        xc = _unpack(xa[_rows(c, TA // 2), :])
        for g in range(NG):
            accumulate_kv(xc, g, key_features(xc, g))
        return 0

    lax.fori_loop(1, NCA, phase1, 0)

    wq_cp.wait()
    cre_cp.wait()
    cim_cp.wait()
    k2r = lam[9]
    k2i = lam[10]
    kni = -k2i
    rr = lax.broadcasted_iota(jnp.int32, (48, 2 * PR), 0)
    cc = lax.broadcasted_iota(jnp.int32, (48, 2 * PR), 1)
    diag = jnp.where(rr < PR, rr // DH, (rr - PR) // 4) == (cc % 2)
    zero = pltpu.bitcast(carry[0], U32)
    for g in range(NG):
        packed = fold(0, g)
        for i, r in enumerate(range(GR * g, GR * (g + 1), 16)):
            tie = packed[i] & zero
            c_r = _unpack2(cre[pl.ds(r // 2, 8), :] | tie)
            c_i = _unpack2(cim[pl.ds(r // 2, 8), :] | tie)
            cp[pl.ds(r // 2, 8), 0:D] = _pack2(*[c_r[i] * k2r - c_i[i] * k2i for i in range(2)])
            cp[pl.ds(r // 2, 8), D:2 * D] = _pack2(*[c_r[i] * kni - c_i[i] * k2r for i in range(2)])
        for j in range(4 * g, 4 * g + 4):
            kvm[j] = _pack(jnp.where(diag, kv[j], 0.0))
    bre_cp.wait()
    bim_cp.wait()

    sub = lax.broadcasted_iota(jnp.int32, (8, 128), 0)

    def phase_b(c, _):
        slot = c

        @_when(c + 1 < NCB)
        def _():
            for d in xb_cp(c + 1):
                d.start()

        @_when(c == 0)
        def _():
            wo_cp.start()

        whole = xb.at[:, _rows(c, TB // 2), :]
        cp_in(whole, whole, sem_xb.at[c]).wait()

        base = c * (TB // 2)
        for b in range(TB // BLK):
            for lt in range(LT):
                pieces = []
                for j in range(4):
                    pieces.extend(_unpack2(xb[lt, pl.ds(base + 32 * b + j, 8, stride=4), :]))
                xperm[pl.ds(BLK // 2 * b, BLK // 2), 128 * lt:128 * (lt + 1)] = (
                    _pack(jnp.concatenate(pieces, axis=0)))
        xp = _unpack(xperm[...])
        ubuf[0] = _dot(xp, _unpack(bre[...]), NT)
        ubuf[1] = _dot(xp, _unpack(bim[...]), NT)
        st = [(carry[0, :, 128 * lt:128 * (lt + 1)], carry[1, :, 128 * lt:128 * (lt + 1)]) for lt in range(LT)]
        for b in range(TB // BLK):
            for lt in range(LT):
                ls = slice(128 * lt, 128 * (lt + 1))
                l1 = (lam[0, :, ls], lam[1, :, ls])
                l8 = [(lam[2 + 2 * k, :, ls], lam[3 + 2 * k, :, ls]) for k in range(3)]
                pr, pi = st[lt]
                def u(i):
                    return (ubuf[0, pl.ds(BLK * b + 8 * i, 8), ls], ubuf[1, pl.ds(BLK * b + 8 * i, 8), ls])
                hr, hi = u(0)
                for i in range(1, 8):
                    hr, hi = _cmul(l1[0], l1[1], hr, hi)
                    ur, ui = u(i)
                    hr, hi = hr + ur, hi + ui
                sr = jnp.where(sub == 0, pltpu.roll(pr, 1, 0), pltpu.roll(hr, 1, 0))
                si = jnp.where(sub == 0, pltpu.roll(pi, 1, 0), pltpu.roll(hi, 1, 0))
                for k, sh in enumerate((1, 2, 4)):
                    tr = jnp.where(sub >= sh, pltpu.roll(sr, sh, 0), 0.0)
                    ti = jnp.where(sub >= sh, pltpu.roll(si, sh, 0), 0.0)
                    tr, ti = _cmul(l8[k][0], l8[k][1], tr, ti)
                    sr, si = sr + tr, si + ti
                hr, hi = sr, si
                hs = []
                for i in range(8):
                    hr, hi = _cmul(l1[0], l1[1], hr, hi)
                    ur, ui = u(i)
                    hr, hi = hr + ur, hi + ui
                    hs.append((hr, hi))
                st[lt] = (hr, hi)
                for j in range(4):
                    hbuf[lt, pl.ds(32 * b + j, 8, stride=4), :] = _pack2(hs[2 * j][0], hs[2 * j + 1][0])
                    hbuf[LT + lt, pl.ds(32 * b + j, 8, stride=4), :] = _pack2(hs[2 * j][1], hs[2 * j + 1][1])
        for lt in range(LT):
            carry[0, :, 128 * lt:128 * (lt + 1)] = st[lt][0]
            carry[1, :, 128 * lt:128 * (lt + 1)] = st[lt][1]
        hcat = jnp.concatenate([_unpack(hbuf[k]) for k in range(2 * LT)], axis=1)
        xc = jnp.concatenate([_unpack(xb[lt, _rows(c, TB // 2), :]) for lt in range(LT)], axis=1)
        ob[slot] = _dot(hcat, _unpack(cp[...]), NT) + xc.astype(F32) * lam[8, 0:1, :]
        ob_cp(c, slot).start()
        return 0

    lax.fori_loop(0, NCB, phase_b, 0)

    wo_cp.wait()

    def phase2(c, _):
        slot = c

        xq = _unpack(xa[_rows(c, TQ // 2), :])
        subt = lax.broadcasted_iota(jnp.int32, (8, TQ), 0)
        ots = []
        for g in range(NG):
            pq = _dot(wrows(0, g), xq, NT)
            for j in range(4):
                phi = _feature_map(pq[PR * j:PR * (j + 1)])
                nd = _dot(_unpack(kvm[4 * g + j]), phi, NN)
                rd = _recip(nd[PR:] + 1e-6)
                sw = pltpu.roll(rd, 4, 0)
                r0 = jnp.where(subt < 4, rd, sw)
                r1 = jnp.where(subt < 4, sw, rd)
                ots.append(nd[:PR] * jnp.concatenate([r0, r0, rd, r1, r1], axis=0))
        ot = jnp.concatenate(ots, axis=0)
        ts = TQ // NSUB
        for j in range(NSUB):
            a = _dot(ot[:, j * ts:(j + 1) * ts].T.astype(BF16), _unpack(wo[...]), NN)
            oa[slot, pl.ds(j * ts, ts), :] = a.astype(BF16).astype(F32)
            oa_cp(c, slot, j).start()
        return 0

    lax.fori_loop(0, NCQ, phase2, 0)

    for c in range(NCB):
        ob_cp(c, c).wait()
    for c in range(NCQ):
        for j in range(NSUB):
            oa_cp(c, c, j).wait()


@jax.jit
def pallas_concat_heads__linear_kernel_hedgehog__ssm_conv_s5__prompt_kernel(
    A_x: jax.Array,
    A_wqkv: jax.Array,
    A_w_phi: jax.Array,
    A_wo: jax.Array,
    B_x: jax.Array,
    B_Lambda_re: jax.Array,
    B_Lambda_im: jax.Array,
    B_B_re: jax.Array,
    B_B_im: jax.Array,
    B_C_re: jax.Array,
    B_C_im: jax.Array,
    B_log_dt: jax.Array,
    B_Dskip: jax.Array,
):
    any_spec = pl.BlockSpec(memory_space=pl.ANY)
    vm = pltpu.VMEM
    scratch = [
        vm((S // 2, D), U32),
        vm((LT, S // 2, 128), U32),
        vm((3, D // 2, D), U32),
        vm((D // 2, D), U32),
        vm((D // 2, D), U32),
        vm((D // 2, D), U32),
        vm((D // 2, D), U32),
        vm((D // 2, D), U32),
        vm((DH, DH, H), BF16),
        [vm((D,), BF16) for _ in range(4)],
        vm((D, 128), F32),
        vm((3, D // 2, D), U32),
        vm((D // 2, 2 * D), U32),
        vm((11, 8, D), F32),
        vm((NP, 48, 2 * PR), F32),
        vm((NP, 24, 2 * PR), U32),
        vm((TB // 2, D), U32),
        vm((2, TB, D), F32),
        vm((2 * LT, TB // 2, 128), U32),
        vm((2, 8, D), F32),
        vm((NCB, TB, D), F32),
        vm((NCQ, TQ, D), F32),
        pltpu.SemaphoreType.DMA((13,)),
        pltpu.SemaphoreType.DMA((2,)),
        pltpu.SemaphoreType.DMA((NCA,)),
        pltpu.SemaphoreType.DMA((NCB,)),
        pltpu.SemaphoreType.DMA((2,)),
    ]
    out = pl.pallas_call(
        _kernel,
        out_shape=jax.ShapeDtypeStruct((S, 2 * D), F32),
        in_specs=[any_spec] * 13,
        out_specs=any_spec,
        scratch_shapes=scratch,
        compiler_params=pltpu.CompilerParams(vmem_limit_bytes=100 * 1024 * 1024),
    )(A_x.reshape(S, D), A_wqkv, A_w_phi.transpose(1, 2, 0), A_wo, B_x.reshape(S, D), B_Lambda_re, B_Lambda_im,
      B_B_re, B_B_im, B_C_re, B_C_im, B_log_dt, B_Dskip)
    return out.reshape(1, S, 2 * D)
```
